```python
import jax
import jax.numpy as jnp

def _softmax(x, axis=-1):
    return jax.nn.softmax(x, axis=axis)
def _gelu(x):
    return jax.nn.gelu(x, approximate=True)
def _silu(x):
    return jax.nn.silu(x)
def _sigmoid(x):
    return jax.nn.sigmoid(x)
def _layernorm(x, axis=-1, eps=1e-5):
    m = jnp.mean(x, axis=axis, keepdims=True)
    v = jnp.var(x, axis=axis, keepdims=True)
    return (x - m) / jnp.sqrt(v + eps)
def _scatter_add(tgt, idx, src, axis=0):
    return tgt.at[idx].add(src)
def _segment_sum(src, seg, n):
    return jax.ops.segment_sum(src, seg, n)
class _Rng:
    def __init__(self, key):
        self._k = key
    def _next(self):
        self._k, sub = jax.random.split(self._k)
        return sub
    def normal(self, shape):
        return jax.random.normal(self._next(), shape, dtype=jnp.bfloat16)
    def randint(self, lo, hi, shape):
        return jax.random.randint(self._next(), shape, lo, hi, dtype=jnp.int32)
    def uniform(self, shape, lo=0.0, hi=1.0):
        return jax.random.uniform(self._next(), shape, jnp.bfloat16, lo, hi)
    def permutation(self, n):
        return jax.random.permutation(self._next(), n)


kernel_name = 'sequential_preLN__grouped_kv_mqa__glu_gated_swiglu__prompt'

def _fwd_setup_inputs():
    _rng = _Rng(jax.random.key(int.from_bytes(__import__("os").urandom(4), "little")))
    _w = (lambda a: (lambda t: t.astype(jnp.bfloat16) if jnp.issubdtype(t.dtype, jnp.floating) else t)(jnp.asarray(a)))
    def _A_setup():
        B, S, D, H = 1, 2048, 512, 32
        Dh = D // H
        return {
            "x": _w((lambda *s: _rng.normal(s) * 0.05)(B, S, D)),
            "wq": _w((lambda *s: _rng.normal(s) * 0.05)(D, H * Dh)),
            "wk": _w((lambda *s: _rng.normal(s) * 0.05)(D, Dh)),
            "wv": _w((lambda *s: _rng.normal(s) * 0.05)(D, Dh)),
            "wo": _w((lambda *s: _rng.normal(s) * 0.05)(H * Dh, D)),
        }
    _A_in = _A_setup()

    def _B_setup():
        B, S, D, F = 1, 2048, 512, 1376
        return {
            "x": _w((lambda *s: _rng.normal(s) * 0.05)(B, S, D)),
            "w1": _w((lambda *s: _rng.normal(s) * 0.05)(D, F) * (2.0 / D) ** 0.5),
            "w3": _w((lambda *s: _rng.normal(s) * 0.05)(D, F) * (2.0 / D) ** 0.5),
            "w2": _w((lambda *s: _rng.normal(s) * 0.05)(F, D) * (2.0 / F) ** 0.5),
        }
    _B_in = _B_setup()

    return {
        "A_x": _A_in["x"],
        "A_wq": _A_in["wq"],
        "A_wk": _A_in["wk"],
        "A_wv": _A_in["wv"],
        "A_wo": _A_in["wo"],
        "B_x": _B_in["x"],
        "B_w1": _B_in["w1"],
        "B_w3": _B_in["w3"],
        "B_w2": _B_in["w2"],
    }

def _fwd_reference(A_x, A_wq, A_wk, A_wv, A_wo, B_x, B_w1, B_w3, B_w2):
    def _A_ref(x, wq, wk, wv, wo):
        B, S, D = x.shape
        H = 32
        Dh = D // H
        q = (lambda x, *d: x.transpose(*d))((x @ wq).reshape(B, S, H, Dh), 0, 2, 1, 3)
        k = x @ wk
        v = x @ wv
        scores = jnp.einsum("bhqd,bkd->bhqk", q, k) * (Dh ** -0.5)
        p = _softmax(scores, axis=-1)
        o = jnp.einsum("bhqk,bkd->bhqd", p, v)
        return (lambda x, *d: x.transpose(*d))(o, 0, 2, 1, 3).reshape(B, S, H * Dh) @ wo

    def _B_ref(x, w1, w3, w2):
        gate = jnp.einsum("bsd,df->bsf", x, w1)
        up = jnp.einsum("bsd,df->bsf", x, w3)
        h = _silu(gate) * up
        out = jnp.einsum("bsf,fd->bsd", h, w2)
        return out

    x = A_x
    h = x + _A_ref(_layernorm(x, axis=-1), A_wq, A_wk, A_wv, A_wo)
    h2 = h + _B_ref(_layernorm(h, axis=-1), B_w1, B_w3, B_w2)
    return h2


def setup_inputs():
    _inp = _fwd_setup_inputs()
    _gk = jax.random.fold_in(jax.random.key(int.from_bytes(__import__("os").urandom(4), "little")), 2**31 - 1)
    _shapes = [[1, 2048, 512]]
    _dtypes = ['bfloat16']
    _gks = jax.random.split(_gk, len(_shapes))
    _gs = [jax.random.normal(k, s, dtype=jnp.dtype(d)) * 0.05 for k, s, d in zip(_gks, _shapes, _dtypes)]
    _inp["grad_out"] = _gs[0]
    return _inp

def reference(A_x, A_wq, A_wk, A_wv, A_wo, B_w1, B_w3, B_w2, B_x, grad_out):
    _const = dict(B_x=B_x)
    def _f(*_d):
        return _fwd_reference(**{'A_x': _d[0], 'A_wq': _d[1], 'A_wk': _d[2], 'A_wv': _d[3], 'A_wo': _d[4], 'B_w1': _d[5], 'B_w3': _d[6], 'B_w2': _d[7], **_const})
    _out, _vjp = jax.vjp(_f, A_x, A_wq, A_wk, A_wv, A_wo, B_w1, B_w3, B_w2)
    _grads = _vjp(grad_out)
    _out0 = jnp.asarray(_out)
    return (_out0, *[jnp.asarray(_g) for _g in _grads])
```

```python
import jax
import jax.numpy as jnp
import jax.experimental.pallas as pl
import jax.experimental.pallas.tpu as pltpu

S, D, H, Dh, F = 2048, 512, 32, 16, 1376
BQ = 128
NQ = S // BQ
CK = 256
NC = S // CK
EPS = 1e-5
SCALE = Dh ** -0.5


def _ln_fwd(x32):
    mu = jnp.mean(x32, axis=-1, keepdims=True)
    xc = x32 - mu
    var = jnp.mean(xc * xc, axis=-1, keepdims=True)
    r = jax.lax.rsqrt(var + EPS)
    return xc * r, r


def _ln_bwd(dn, n, r):
    m1 = jnp.mean(dn, axis=-1, keepdims=True)
    m2 = jnp.mean(dn * n, axis=-1, keepdims=True)
    return r * (dn - m1 - n * m2)


def _nt(a, b):
    return jax.lax.dot_general(a, b, (((1,), (1,)), ((), ())), preferred_element_type=jnp.float32)


def _tn(a, b):
    return jax.lax.dot_general(a, b, (((0,), (0,)), ((), ())), preferred_element_type=jnp.float32)


def _nn(a, b):
    return jnp.dot(a, b, preferred_element_type=jnp.float32)


def _kernel(x_ref, g_ref, wq_ref, wk_ref, wv_ref, wo_ref, w1_ref, w3_ref, w2_ref,
            out_ref, dx_ref, dwq_ref, dwk_ref, dwv_ref, dwo_ref, dw1_ref, dw3_ref, dw2_ref,
            n1_s, r1_s, dh_s, dn1_s, k_s, v_s, kt_s, vt_s, wqt_s,
            qt_s, ot_s, dot_s, dqt_s, p_s, s_a, s_b, m_a, m_b, l_s, dkt_s, dvt_s,
            dwqt_acc, dwo_acc, dw1_acc, dw3_acc, dw2_acc):
    i = pl.program_id(0)
    rows = pl.ds(pl.multiple_of(i * BQ, BQ), BQ)

    @pl.when(i == 0)
    def _():
        def ln_chunk(c, carry):
            rs = pl.ds(pl.multiple_of(c * BQ, BQ), BQ)
            n, r = _ln_fwd(x_ref[rs, :].astype(jnp.float32))
            n1_s[rs, :] = n.astype(jnp.bfloat16)
            r1_s[rs, :] = r
            return carry
        jax.lax.fori_loop(0, NQ, ln_chunk, 0)
        k = _nn(n1_s[...], wk_ref[...]).astype(jnp.bfloat16)
        v = _nn(n1_s[...], wv_ref[...]).astype(jnp.bfloat16)
        k_s[...] = k
        v_s[...] = v
        kt_s[...] = k.T
        vt_s[...] = v.T
        wqt_s[...] = wq_ref[...].T
        dkt_s[...] = jnp.zeros_like(dkt_s)
        dvt_s[...] = jnp.zeros_like(dvt_s)
        dwqt_acc[...] = jnp.zeros_like(dwqt_acc)
        dwo_acc[...] = jnp.zeros_like(dwo_acc)
        dw1_acc[...] = jnp.zeros_like(dw1_acc)
        dw3_acc[...] = jnp.zeros_like(dw3_acc)
        dw2_acc[...] = jnp.zeros_like(dw2_acc)

    x_blk = x_ref[rows, :].astype(jnp.float32)
    n1_blk = n1_s[rows, :]

    qt_s[...] = (_nt(wqt_s[...], n1_blk) * SCALE).astype(jnp.bfloat16)

    def qk(h, s_ref, m_ref):
        qt = qt_s[pl.ds(pl.multiple_of(h * Dh, Dh), Dh), :]
        sT = _nn(k_s[...], qt)
        s_ref[...] = sT
        m_ref[...] = jnp.max(sT, axis=0, keepdims=True)

    def fused_fwd(hn, sn_ref, mn_ref, h, s_ref, m_ref):
        qtn = qt_s[pl.ds(pl.multiple_of(hn * Dh, Dh), Dh), :]
        m = m_ref[...]
        mn = jnp.full((1, BQ), -jnp.inf, jnp.float32)
        l = jnp.zeros((1, BQ), jnp.float32)
        oT = jnp.zeros((Dh, BQ), jnp.float32)
        for c in range(NC):
            ks = slice(c * CK, (c + 1) * CK)
            sT = _nn(k_s[ks, :], qtn)
            sn_ref[ks, :] = sT
            mn = jnp.maximum(mn, jnp.max(sT, axis=0, keepdims=True))
            p = jnp.exp(s_ref[ks, :] - m)
            l = l + jnp.sum(p, axis=0, keepdims=True)
            p_s[h, ks, :] = p.astype(jnp.bfloat16)
            oT = oT + _nn(vt_s[:, ks], p_s[h, ks, :])
        mn_ref[...] = mn
        linv = 1.0 / l
        l_s[h] = linv
        ot_s[pl.ds(pl.multiple_of(h * Dh, Dh), Dh), :] = oT * linv

    qk(0, s_a, m_a)

    def fwd_body(j, c):
        h0 = 2 * j; h1 = 2 * j + 1
        hn = jnp.minimum(h1 + 1, H - 1)
        fused_fwd(h1, s_b, m_b, h0, s_a, m_a)
        fused_fwd(hn, s_a, m_a, h1, s_b, m_b)
        return c
    jax.lax.fori_loop(0, H // 2, fwd_body, 0)

    o_bf = ot_s[...].astype(jnp.bfloat16)
    a = _tn(o_bf, wo_ref[...])
    h = x_blk + a
    n2, r2 = _ln_fwd(h)
    n2_bf = n2.astype(jnp.bfloat16)
    g_ = _nn(n2_bf, w1_ref[...])
    u_ = _nn(n2_bf, w3_ref[...])
    sig = jax.nn.sigmoid(g_)
    sg = g_ * sig
    f_ = (sg * u_).astype(jnp.bfloat16)
    y = _nn(f_, w2_ref[...])
    out_ref[...] = (h + y).astype(out_ref.dtype)

    G = g_ref[rows, :]
    G32 = G.astype(jnp.float32)
    dw2_acc[...] += _tn(f_, G)
    df = _nt(G, w2_ref[...])
    du = df * sg
    dg = df * u_ * (sig * (1.0 + g_ * (1.0 - sig)))
    dg_bf = dg.astype(jnp.bfloat16)
    du_bf = du.astype(jnp.bfloat16)
    dw1_acc[...] += _tn(n2_bf, dg_bf)
    dw3_acc[...] += _tn(n2_bf, du_bf)
    dn2 = _nt(dg_bf, w1_ref[...]) + _nt(du_bf, w3_ref[...])
    dh = G32 + _ln_bwd(dn2, n2, r2)
    da = dh.astype(jnp.bfloat16)
    dwo_acc[...] += _nn(o_bf, da)
    dot_s[...] = _nt(wo_ref[...], da).astype(jnp.bfloat16)
    dh_s[rows, :] = dh

    def dpk(h, s_ref):
        doT = dot_s[pl.ds(pl.multiple_of(h * Dh, Dh), Dh), :]
        s_ref[...] = _nn(v_s[...], doT)

    def fused_bwd(hn, sn_ref, h, s_ref):
        hs = pl.multiple_of(h * Dh, Dh)
        doTn = dot_s[pl.ds(pl.multiple_of(hn * Dh, Dh), Dh), :]
        qt = qt_s[pl.ds(hs, Dh), :].astype(jnp.float32)
        doT = dot_s[pl.ds(hs, Dh), :].astype(jnp.float32)
        oT = ot_s[pl.ds(hs, Dh), :]
        delta = jnp.sum(doT * oT, axis=0, keepdims=True)
        linv = l_s[h]
        qtl = (qt * linv).astype(jnp.bfloat16)
        dol = (doT * linv).astype(jnp.bfloat16)
        dqT = jnp.zeros((Dh, BQ), jnp.float32)
        for c in range(NC):
            ks = slice(c * CK, (c + 1) * CK)
            sn_ref[ks, :] = _nn(v_s[ks, :], doTn)
            ds = (p_s[h, ks, :].astype(jnp.float32) * (s_ref[ks, :] - delta)).astype(jnp.bfloat16)
            dqT = dqT + _nn(kt_s[:, ks], ds)
            dkt_s[:, ks] += _nt(qtl, ds)
            dvt_s[:, ks] += _nt(dol, p_s[h, ks, :])
        dqt_s[pl.ds(hs, Dh), :] = dqT * (linv * SCALE)

    dpk(0, s_a)

    def bwd_body(j, c):
        h0 = 2 * j; h1 = 2 * j + 1
        hn = jnp.minimum(h1 + 1, H - 1)
        fused_bwd(h1, s_b, h0, s_a)
        fused_bwd(hn, s_a, h1, s_b)
        return c
    jax.lax.fori_loop(0, H // 2, bwd_body, 0)

    dqt_bf = dqt_s[...].astype(jnp.bfloat16)
    dwqt_acc[...] += _nn(dqt_bf, n1_blk)
    dn1_s[rows, :] = jax.lax.dot_general(dqt_bf, wq_ref[...], (((0,), (1,)), ((), ())), preferred_element_type=jnp.float32)

    @pl.when(i == NQ - 1)
    def _():
        dkt_bf = dkt_s[...].astype(jnp.bfloat16)
        dvt_bf = dvt_s[...].astype(jnp.bfloat16)
        dn1_kv = jax.lax.dot_general(dkt_bf, wk_ref[...], (((0,), (1,)), ((), ())),
                                     preferred_element_type=jnp.float32) + \
                 jax.lax.dot_general(dvt_bf, wv_ref[...], (((0,), (1,)), ((), ())),
                                     preferred_element_type=jnp.float32)
        def dx_chunk(c, carry):
            rs = pl.ds(pl.multiple_of(c * BQ, BQ), BQ)
            n = n1_s[rs, :].astype(jnp.float32)
            dn = dn1_s[rs, :] + dn1_kv_chunk(c)
            dx_ref[rs, :] = (dh_s[rs, :] + _ln_bwd(dn, n, r1_s[rs, :])).astype(dx_ref.dtype)
            return carry

        def dn1_kv_chunk(c):
            cs = pl.ds(pl.multiple_of(c * BQ, BQ), BQ)
            dk = dkt_s[:, cs].astype(jnp.bfloat16)
            dv = dvt_s[:, cs].astype(jnp.bfloat16)
            return jax.lax.dot_general(dk, wk_ref[...], (((0,), (1,)), ((), ())),
                                       preferred_element_type=jnp.float32) + \
                   jax.lax.dot_general(dv, wv_ref[...], (((0,), (1,)), ((), ())),
                                       preferred_element_type=jnp.float32)
        for c in range(NQ):
            dx_chunk(c, 0)
        dwk_ref[...] = _nn(dkt_bf, n1_s[...]).T.astype(dwk_ref.dtype)
        dwv_ref[...] = _nn(dvt_bf, n1_s[...]).T.astype(dwv_ref.dtype)
        dwq_ref[...] = dwqt_acc[...].T.astype(dwq_ref.dtype)
        dwo_ref[...] = dwo_acc[...].astype(dwo_ref.dtype)
        dw1_ref[...] = dw1_acc[...].astype(dw1_ref.dtype)
        dw3_ref[...] = dw3_acc[...].astype(dw3_ref.dtype)
        dw2_ref[...] = dw2_acc[...].astype(dw2_ref.dtype)


@jax.jit
def pallas_sequential_preLN__grouped_kv_mqa__glu_gated_swiglu__prompt_kernel(
    A_x: jax.Array,
    A_wq: jax.Array,
    A_wk: jax.Array,
    A_wv: jax.Array,
    A_wo: jax.Array,
    B_x: jax.Array,
    B_w1: jax.Array,
    B_w3: jax.Array,
    B_w2: jax.Array,
    grad_out: jax.Array,
):
    x = A_x.reshape(S, D)
    g = grad_out.reshape(S, D)
    full = lambda shape: pl.BlockSpec(shape, lambda i: (0,) * len(shape), pipeline_mode=pl.Buffered(1))
    bf = jnp.bfloat16
    f32 = jnp.float32
    out_shape = [
        jax.ShapeDtypeStruct((S, D), bf),
        jax.ShapeDtypeStruct((S, D), bf),
        jax.ShapeDtypeStruct((D, H * Dh), bf),
        jax.ShapeDtypeStruct((D, Dh), bf),
        jax.ShapeDtypeStruct((D, Dh), bf),
        jax.ShapeDtypeStruct((H * Dh, D), bf),
        jax.ShapeDtypeStruct((D, F), bf),
        jax.ShapeDtypeStruct((D, F), bf),
        jax.ShapeDtypeStruct((F, D), bf),
    ]
    fullout = lambda shape: pl.BlockSpec(shape, lambda i: (0,) * len(shape))
    outs = pl.pallas_call(
        _kernel,
        grid=(NQ,),
        in_specs=[
            full((S, D)), full((S, D)), full((D, H * Dh)), full((D, Dh)), full((D, Dh)),
            full((H * Dh, D)), full((D, F)), full((D, F)), full((F, D)),
        ],
        out_specs=[
            pl.BlockSpec((BQ, D), lambda i: (i, 0)),
            fullout((S, D)), fullout((D, H * Dh)), fullout((D, Dh)), fullout((D, Dh)),
            fullout((H * Dh, D)), fullout((D, F)), fullout((D, F)), fullout((F, D)),
        ],
        out_shape=out_shape,
        scratch_shapes=[
            pltpu.VMEM((S, D), bf),
            pltpu.VMEM((S, 1), f32),
            pltpu.VMEM((S, D), f32),
            pltpu.VMEM((S, D), f32),
            pltpu.VMEM((S, Dh), bf),
            pltpu.VMEM((S, Dh), bf),
            pltpu.VMEM((Dh, S), bf),
            pltpu.VMEM((Dh, S), bf),
            pltpu.VMEM((H * Dh, D), bf),
            pltpu.VMEM((H * Dh, BQ), bf),
            pltpu.VMEM((H * Dh, BQ), f32),
            pltpu.VMEM((H * Dh, BQ), bf),
            pltpu.VMEM((H * Dh, BQ), f32),
            pltpu.VMEM((H, S, BQ), bf),
            pltpu.VMEM((S, BQ), f32),
            pltpu.VMEM((S, BQ), f32),
            pltpu.VMEM((1, BQ), f32),
            pltpu.VMEM((1, BQ), f32),
            pltpu.VMEM((H, 1, BQ), f32),
            pltpu.VMEM((Dh, S), f32),
            pltpu.VMEM((Dh, S), f32),
            pltpu.VMEM((H * Dh, D), f32),
            pltpu.VMEM((H * Dh, D), f32),
            pltpu.VMEM((D, F), f32),
            pltpu.VMEM((D, F), f32),
            pltpu.VMEM((F, D), f32),
        ],
        compiler_params=pltpu.CompilerParams(
            dimension_semantics=("arbitrary",),
            vmem_limit_bytes=110 * 1024 * 1024,
        ),
    )(x, g, A_wq, A_wk, A_wv, A_wo, B_w1, B_w3, B_w2)
    out, dx, dwq, dwk, dwv, dwo, dw1, dw3, dw2 = outs
    return (out.reshape(1, S, D), dx.reshape(1, S, D), dwq, dwk, dwv, dwo, dw1, dw3, dw2)
```

```python
import contextlib
import jax
import jax.numpy as jnp
import jax.experimental.pallas as pl
import jax.experimental.pallas.tpu as pltpu

S, D, H, Dh, F = 2048, 512, 32, 16, 1376
BQ = 256
NQ = S // BQ
CK = 128
NC = S // CK
EPS = 1e-5
SCALE = Dh ** -0.5
_SCOPES = False


def _scope(name):
    return jax.named_scope(name) if _SCOPES else contextlib.nullcontext()


def _ln_fwd(x32):
    mu = jnp.mean(x32, axis=-1, keepdims=True)
    xc = x32 - mu
    var = jnp.mean(xc * xc, axis=-1, keepdims=True)
    r = jax.lax.rsqrt(var + EPS)
    return xc * r, r


def _ln_bwd(dn, n, r):
    m1 = jnp.mean(dn, axis=-1, keepdims=True)
    m2 = jnp.mean(dn * n, axis=-1, keepdims=True)
    return r * (dn - m1 - n * m2)


def _nt(a, b):
    return jax.lax.dot_general(a, b, (((1,), (1,)), ((), ())), preferred_element_type=jnp.float32)


def _tn(a, b):
    return jax.lax.dot_general(a, b, (((0,), (0,)), ((), ())), preferred_element_type=jnp.float32)


def _nn(a, b):
    return jnp.dot(a, b, preferred_element_type=jnp.float32)


def _kernel(x_ref, g_ref, wq_ref, wk_ref, wv_ref, wo_ref, w1_ref, w3_ref, w2_ref,
            out_ref, dx_ref, dwq_ref, dwk_ref, dwv_ref, dwo_ref, dw1_ref, dw3_ref, dw2_ref,
            n1_s, r1_s, dh_s, dn1_s, k_s, v_s, kt_s, vt_s, wqt_s,
            qt_s, ot_s, dot_s, dqt_s, p_s, s_a, s_b, m_a, m_b, l_s, dkt_s, dvt_s,
            dwqt_acc, dwo_acc, dw1_acc, dw3_acc, dw2_acc):
    i = pl.program_id(0)
    rows = pl.ds(pl.multiple_of(i * BQ, BQ), BQ)

    with _scope('prologue'):
        @pl.when(i == 0)
        def _():
            def ln_chunk(c, carry):
                rs = pl.ds(pl.multiple_of(c * BQ, BQ), BQ)
                n, r = _ln_fwd(x_ref[rs, :].astype(jnp.float32))
                n1_s[rs, :] = n.astype(jnp.bfloat16)
                r1_s[rs, :] = r
                return carry
            jax.lax.fori_loop(0, NQ, ln_chunk, 0)
            k = _nn(n1_s[...], wk_ref[...]).astype(jnp.bfloat16)
            v = _nn(n1_s[...], wv_ref[...]).astype(jnp.bfloat16)
            k_s[...] = k
            v_s[...] = v
            kt_s[...] = k.T
            vt_s[...] = v.T
            wqt_s[...] = wq_ref[...].T
            dkt_s[...] = jnp.zeros_like(dkt_s)
            dvt_s[...] = jnp.zeros_like(dvt_s)
            dwqt_acc[...] = jnp.zeros_like(dwqt_acc)
            dwo_acc[...] = jnp.zeros_like(dwo_acc)
            dw1_acc[...] = jnp.zeros_like(dw1_acc)
            dw3_acc[...] = jnp.zeros_like(dw3_acc)
            dw2_acc[...] = jnp.zeros_like(dw2_acc)

    with _scope('qproj'):
        x_blk = x_ref[rows, :].astype(jnp.float32)
        n1_blk = n1_s[rows, :]

        qt_s[...] = (_nt(wqt_s[...], n1_blk) * SCALE).astype(jnp.bfloat16)

    with _scope('attn_fwd'):
        def qk(h, s_ref, m_ref):
            qt = qt_s[pl.ds(pl.multiple_of(h * Dh, Dh), Dh), :]
            sT = _nn(k_s[...], qt)
            s_ref[...] = sT
            m_ref[...] = jnp.max(sT, axis=0, keepdims=True)

        def fused_fwd(hn, sn_ref, mn_ref, h, s_ref, m_ref):
            qtn = qt_s[pl.ds(pl.multiple_of(hn * Dh, Dh), Dh), :]
            m = m_ref[...]
            mn = jnp.full((1, BQ), -jnp.inf, jnp.float32)
            l = jnp.zeros((1, BQ), jnp.float32)
            oT = jnp.zeros((Dh, BQ), jnp.float32)
            for c in range(NC):
                ks = slice(c * CK, (c + 1) * CK)
                sT = _nn(k_s[ks, :], qtn)
                sn_ref[ks, :] = sT
                mn = jnp.maximum(mn, jnp.max(sT, axis=0, keepdims=True))
                p = jnp.exp(s_ref[ks, :] - m)
                l = l + jnp.sum(p, axis=0, keepdims=True)
                p_s[h, ks, :] = p.astype(jnp.bfloat16)
                oT = oT + _nn(vt_s[:, ks], p_s[h, ks, :])
            mn_ref[...] = mn
            linv = 1.0 / l
            l_s[h] = linv
            ot_s[pl.ds(pl.multiple_of(h * Dh, Dh), Dh), :] = oT * linv

        qk(0, s_a, m_a)

        def fwd_body(j, c):
            h0 = 2 * j; h1 = 2 * j + 1
            hn = jnp.minimum(h1 + 1, H - 1)
            fused_fwd(h1, s_b, m_b, h0, s_a, m_a)
            fused_fwd(hn, s_a, m_a, h1, s_b, m_b)
            return c
        jax.lax.fori_loop(0, H // 2, fwd_body, 0)

    with _scope('mlp_fwd'):
        o_bf = ot_s[...].astype(jnp.bfloat16)
        a = _tn(o_bf, wo_ref[...])
        h = x_blk + a
        n2, r2 = _ln_fwd(h)
        n2_bf = n2.astype(jnp.bfloat16)
        g_ = _nn(n2_bf, w1_ref[...])
        u_ = _nn(n2_bf, w3_ref[...])
        sig = jax.nn.sigmoid(g_)
        sg = g_ * sig
        f_ = (sg * u_).astype(jnp.bfloat16)
        y = _nn(f_, w2_ref[...])
        out_ref[...] = (h + y).astype(out_ref.dtype)

    with _scope('mlp_bwd'):
        G = g_ref[rows, :]
        G32 = G.astype(jnp.float32)
        dw2_acc[...] += _tn(f_, G)
        df = _nt(G, w2_ref[...])
        du = df * sg
        dg = df * u_ * (sig * (1.0 + g_ * (1.0 - sig)))
        dg_bf = dg.astype(jnp.bfloat16)
        du_bf = du.astype(jnp.bfloat16)
        dw1_acc[...] += _tn(n2_bf, dg_bf)
        dw3_acc[...] += _tn(n2_bf, du_bf)
        dn2 = _nt(dg_bf, w1_ref[...]) + _nt(du_bf, w3_ref[...])
        dh = G32 + _ln_bwd(dn2, n2, r2)
        da = dh.astype(jnp.bfloat16)
        dwo_acc[...] += _nn(o_bf, da)
        dot_s[...] = _nt(wo_ref[...], da).astype(jnp.bfloat16)
        dh_s[rows, :] = dh

    with _scope('attn_bwd'):
        def dpk(h, s_ref):
            doT = dot_s[pl.ds(pl.multiple_of(h * Dh, Dh), Dh), :]
            s_ref[...] = _nn(v_s[...], doT)

        def fused_bwd(hn, sn_ref, h, s_ref):
            hs = pl.multiple_of(h * Dh, Dh)
            doTn = dot_s[pl.ds(pl.multiple_of(hn * Dh, Dh), Dh), :]
            qt = qt_s[pl.ds(hs, Dh), :].astype(jnp.float32)
            doT = dot_s[pl.ds(hs, Dh), :].astype(jnp.float32)
            oT = ot_s[pl.ds(hs, Dh), :]
            delta = jnp.sum(doT * oT, axis=0, keepdims=True)
            linv = l_s[h]
            qtl = (qt * linv).astype(jnp.bfloat16)
            dol = (doT * linv).astype(jnp.bfloat16)
            dqT = jnp.zeros((Dh, BQ), jnp.float32)
            for c in range(NC):
                ks = slice(c * CK, (c + 1) * CK)
                sn_ref[ks, :] = _nn(v_s[ks, :], doTn)
                ds = (p_s[h, ks, :].astype(jnp.float32) * (s_ref[ks, :] - delta)).astype(jnp.bfloat16)
                dqT = dqT + _nn(kt_s[:, ks], ds)
                dkt_s[:, ks] += _nt(qtl, ds)
                dvt_s[:, ks] += _nt(dol, p_s[h, ks, :])
            dqt_s[pl.ds(hs, Dh), :] = dqT * (linv * SCALE)

        dpk(0, s_a)

        def bwd_body(j, c):
            h0 = 2 * j; h1 = 2 * j + 1
            hn = jnp.minimum(h1 + 1, H - 1)
            fused_bwd(h1, s_b, h0, s_a)
            fused_bwd(hn, s_a, h1, s_b)
            return c
        jax.lax.fori_loop(0, H // 2, bwd_body, 0)

    with _scope('wgrad_q'):
        dqt_bf = dqt_s[...].astype(jnp.bfloat16)
        dwqt_acc[...] += _nn(dqt_bf, n1_blk)
        dn1_s[rows, :] = jax.lax.dot_general(dqt_bf, wq_ref[...], (((0,), (1,)), ((), ())), preferred_element_type=jnp.float32)

    with _scope('epilogue'):
        @pl.when(i == NQ - 1)
        def _():
            dkt_bf = dkt_s[...].astype(jnp.bfloat16)
            dvt_bf = dvt_s[...].astype(jnp.bfloat16)
            dn1_kv = jax.lax.dot_general(dkt_bf, wk_ref[...], (((0,), (1,)), ((), ())),
                                         preferred_element_type=jnp.float32) + \
                     jax.lax.dot_general(dvt_bf, wv_ref[...], (((0,), (1,)), ((), ())),
                                         preferred_element_type=jnp.float32)
            def dx_chunk(c, carry):
                rs = pl.ds(pl.multiple_of(c * BQ, BQ), BQ)
                n = n1_s[rs, :].astype(jnp.float32)
                dn = dn1_s[rs, :] + dn1_kv_chunk(c)
                dx_ref[rs, :] = (dh_s[rs, :] + _ln_bwd(dn, n, r1_s[rs, :])).astype(dx_ref.dtype)
                return carry

            def dn1_kv_chunk(c):
                cs = pl.ds(pl.multiple_of(c * BQ, BQ), BQ)
                dk = dkt_s[:, cs].astype(jnp.bfloat16)
                dv = dvt_s[:, cs].astype(jnp.bfloat16)
                return jax.lax.dot_general(dk, wk_ref[...], (((0,), (1,)), ((), ())),
                                           preferred_element_type=jnp.float32) + \
                       jax.lax.dot_general(dv, wv_ref[...], (((0,), (1,)), ((), ())),
                                           preferred_element_type=jnp.float32)
            for c in range(NQ):
                dx_chunk(c, 0)
            dwk_ref[...] = _nn(dkt_bf, n1_s[...]).T.astype(dwk_ref.dtype)
            dwv_ref[...] = _nn(dvt_bf, n1_s[...]).T.astype(dwv_ref.dtype)
            dwq_ref[...] = dwqt_acc[...].T.astype(dwq_ref.dtype)
            dwo_ref[...] = dwo_acc[...].astype(dwo_ref.dtype)
            dw1_ref[...] = dw1_acc[...].astype(dw1_ref.dtype)
            dw3_ref[...] = dw3_acc[...].astype(dw3_ref.dtype)
            dw2_ref[...] = dw2_acc[...].astype(dw2_ref.dtype)


@jax.jit
def pallas_sequential_preLN__grouped_kv_mqa__glu_gated_swiglu__prompt_kernel(
    A_x: jax.Array,
    A_wq: jax.Array,
    A_wk: jax.Array,
    A_wv: jax.Array,
    A_wo: jax.Array,
    B_x: jax.Array,
    B_w1: jax.Array,
    B_w3: jax.Array,
    B_w2: jax.Array,
    grad_out: jax.Array,
):
    x = A_x.reshape(S, D)
    g = grad_out.reshape(S, D)
    full = lambda shape: pl.BlockSpec(shape, lambda i: (0,) * len(shape), pipeline_mode=pl.Buffered(1))
    bf = jnp.bfloat16
    f32 = jnp.float32
    out_shape = [
        jax.ShapeDtypeStruct((S, D), bf),
        jax.ShapeDtypeStruct((S, D), bf),
        jax.ShapeDtypeStruct((D, H * Dh), bf),
        jax.ShapeDtypeStruct((D, Dh), bf),
        jax.ShapeDtypeStruct((D, Dh), bf),
        jax.ShapeDtypeStruct((H * Dh, D), bf),
        jax.ShapeDtypeStruct((D, F), bf),
        jax.ShapeDtypeStruct((D, F), bf),
        jax.ShapeDtypeStruct((F, D), bf),
    ]
    fullout = lambda shape: pl.BlockSpec(shape, lambda i: (0,) * len(shape))
    outs = pl.pallas_call(
        _kernel,
        grid=(NQ,),
        in_specs=[
            full((S, D)), full((S, D)), full((D, H * Dh)), full((D, Dh)), full((D, Dh)),
            full((H * Dh, D)), full((D, F)), full((D, F)), full((F, D)),
        ],
        out_specs=[
            pl.BlockSpec((BQ, D), lambda i: (i, 0)),
            fullout((S, D)), fullout((D, H * Dh)), fullout((D, Dh)), fullout((D, Dh)),
            fullout((H * Dh, D)), fullout((D, F)), fullout((D, F)), fullout((F, D)),
        ],
        out_shape=out_shape,
        scratch_shapes=[
            pltpu.VMEM((S, D), bf),
            pltpu.VMEM((S, 1), f32),
            pltpu.VMEM((S, D), f32),
            pltpu.VMEM((S, D), f32),
            pltpu.VMEM((S, Dh), bf),
            pltpu.VMEM((S, Dh), bf),
            pltpu.VMEM((Dh, S), bf),
            pltpu.VMEM((Dh, S), bf),
            pltpu.VMEM((H * Dh, D), bf),
            pltpu.VMEM((H * Dh, BQ), bf),
            pltpu.VMEM((H * Dh, BQ), f32),
            pltpu.VMEM((H * Dh, BQ), bf),
            pltpu.VMEM((H * Dh, BQ), f32),
            pltpu.VMEM((H, S, BQ), bf),
            pltpu.VMEM((S, BQ), f32),
            pltpu.VMEM((S, BQ), f32),
            pltpu.VMEM((1, BQ), f32),
            pltpu.VMEM((1, BQ), f32),
            pltpu.VMEM((H, 1, BQ), f32),
            pltpu.VMEM((Dh, S), f32),
            pltpu.VMEM((Dh, S), f32),
            pltpu.VMEM((H * Dh, D), f32),
            pltpu.VMEM((H * Dh, D), f32),
            pltpu.VMEM((D, F), f32),
            pltpu.VMEM((D, F), f32),
            pltpu.VMEM((F, D), f32),
        ],
        compiler_params=pltpu.CompilerParams(
            dimension_semantics=("arbitrary",),
            vmem_limit_bytes=110 * 1024 * 1024,
        ),
    )(x, g, A_wq, A_wk, A_wv, A_wo, B_w1, B_w3, B_w2)
    out, dx, dwq, dwk, dwv, dwo, dw1, dw3, dw2 = outs
    return (out.reshape(1, S, D), dx.reshape(1, S, D), dwq, dwk, dwv, dwo, dw1, dw3, dw2)
```

```python
import contextlib
import jax
import jax.numpy as jnp
import jax.experimental.pallas as pl
import jax.experimental.pallas.tpu as pltpu

S, D, H, Dh, F = 2048, 512, 32, 16, 1376
BQ = 256
NQ = S // BQ
CK = 128
NC = S // CK
EPS = 1e-5
SCALE = Dh ** -0.5
_SCOPES = False


def _scope(name):
    return jax.named_scope(name) if _SCOPES else contextlib.nullcontext()


def _ln_fwd(x32):
    mu = jnp.mean(x32, axis=-1, keepdims=True)
    xc = x32 - mu
    var = jnp.mean(xc * xc, axis=-1, keepdims=True)
    r = jax.lax.rsqrt(var + EPS)
    return xc * r, r


def _ln_bwd(dn, n, r):
    m1 = jnp.mean(dn, axis=-1, keepdims=True)
    m2 = jnp.mean(dn * n, axis=-1, keepdims=True)
    return r * (dn - m1 - n * m2)


def _nt(a, b):
    return jax.lax.dot_general(a, b, (((1,), (1,)), ((), ())), preferred_element_type=jnp.float32)


def _tn(a, b):
    return jax.lax.dot_general(a, b, (((0,), (0,)), ((), ())), preferred_element_type=jnp.float32)


def _nn(a, b):
    return jnp.dot(a, b, preferred_element_type=jnp.float32)


def _kernel(x_ref, g_ref, wq_ref, wk_ref, wv_ref, wo_ref, w1_ref, w3_ref, w2_ref,
            out_ref, dx_ref, dwq_ref, dwk_ref, dwv_ref, dwo_ref, dw1_ref, dw3_ref, dw2_ref,
            n1_s, r1_s, dh_s, dn1_s, k_s, v_s, kt_s, vt_s, wqt_s,
            qt_s, ot_s, dot_s, dqt_s, p_s, s_a, s_b, m_a, m_b, l_s, dkt_s, dvt_s,
            dwqt_acc, dwo_acc, dw1_acc, dw3_acc, dw2_acc):
    i = pl.program_id(0)
    rows = pl.ds(pl.multiple_of(i * BQ, BQ), BQ)

    with _scope('prologue'):
        @pl.when(i == 0)
        def _():
            def ln_chunk(c, carry):
                rs = pl.ds(pl.multiple_of(c * BQ, BQ), BQ)
                n, r = _ln_fwd(x_ref[rs, :].astype(jnp.float32))
                n1_s[rs, :] = n.astype(jnp.bfloat16)
                r1_s[rs, :] = r
                return carry
            jax.lax.fori_loop(0, NQ, ln_chunk, 0)
            k = _nn(n1_s[...], wk_ref[...]).astype(jnp.bfloat16)
            v = _nn(n1_s[...], wv_ref[...]).astype(jnp.bfloat16)
            k_s[...] = k
            v_s[...] = v
            kt_s[...] = k.T
            vt_s[...] = v.T
            wqt_s[...] = wq_ref[...].T
            dkt_s[...] = jnp.zeros_like(dkt_s)
            dvt_s[...] = jnp.zeros_like(dvt_s)
            dwqt_acc[...] = jnp.zeros_like(dwqt_acc)
            dwo_acc[...] = jnp.zeros_like(dwo_acc)
            dw1_acc[...] = jnp.zeros_like(dw1_acc)
            dw3_acc[...] = jnp.zeros_like(dw3_acc)
            dw2_acc[...] = jnp.zeros_like(dw2_acc)

    with _scope('qproj'):
        x_blk = x_ref[rows, :].astype(jnp.float32)
        n1_blk = n1_s[rows, :]

        qt_s[...] = (_nt(wqt_s[...], n1_blk) * SCALE).astype(jnp.bfloat16)

    with _scope('attn_fwd'):
        def qk(h, s_ref, m_ref):
            qt = qt_s[pl.ds(pl.multiple_of(h * Dh, Dh), Dh), :]
            sT = _nn(k_s[...], qt)
            s_ref[...] = sT
            m_ref[...] = jnp.max(jnp.max(sT.reshape(S // 8, 8, BQ), axis=0), axis=0, keepdims=True)

        def fused_fwd(hn, sn_ref, mn_ref, h, s_ref, m_ref):
            qtn = qt_s[pl.ds(pl.multiple_of(hn * Dh, Dh), Dh), :]
            m = m_ref[...]
            mn = jnp.full((8, BQ), -jnp.inf, jnp.float32)
            l8 = jnp.zeros((8, BQ), jnp.float32)
            oT = jnp.zeros((Dh, BQ), jnp.float32)
            for c in range(NC):
                ks = slice(c * CK, (c + 1) * CK)
                sT = _nn(k_s[ks, :], qtn)
                sn_ref[ks, :] = sT
                mn = jnp.maximum(mn, jnp.max(sT.reshape(CK // 8, 8, BQ), axis=0))
                p = jnp.exp(s_ref[ks, :] - m)
                l8 = l8 + jnp.sum(p.reshape(CK // 8, 8, BQ), axis=0)
                pb = p.astype(jnp.bfloat16)
                p_s[h, ks, :] = pb
                oT = oT + _nn(vt_s[:, ks], pb)
            mn_ref[...] = jnp.max(mn, axis=0, keepdims=True)
            linv = 1.0 / jnp.sum(l8, axis=0, keepdims=True)
            l_s[h] = linv
            ot_s[pl.ds(pl.multiple_of(h * Dh, Dh), Dh), :] = oT * linv

        qk(0, s_a, m_a)

        def fwd_body(j, c):
            h0 = 2 * j; h1 = 2 * j + 1
            hn = jnp.minimum(h1 + 1, H - 1)
            fused_fwd(h1, s_b, m_b, h0, s_a, m_a)
            fused_fwd(hn, s_a, m_a, h1, s_b, m_b)
            return c
        jax.lax.fori_loop(0, H // 2, fwd_body, 0)

    with _scope('mlp_fwd'):
        o_bf = ot_s[...].astype(jnp.bfloat16)
        a = _tn(o_bf, wo_ref[...])
        h = x_blk + a
        n2, r2 = _ln_fwd(h)
        n2_bf = n2.astype(jnp.bfloat16)
        g_ = _nn(n2_bf, w1_ref[...])
        u_ = _nn(n2_bf, w3_ref[...])
        sig = jax.nn.sigmoid(g_)
        sg = g_ * sig
        f_ = (sg * u_).astype(jnp.bfloat16)
        y = _nn(f_, w2_ref[...])
        out_ref[...] = (h + y).astype(out_ref.dtype)

    with _scope('mlp_bwd'):
        G = g_ref[rows, :]
        G32 = G.astype(jnp.float32)
        dw2_acc[...] += _tn(f_, G)
        df = _nt(G, w2_ref[...])
        du = df * sg
        dg = df * u_ * (sig * (1.0 + g_ * (1.0 - sig)))
        dg_bf = dg.astype(jnp.bfloat16)
        du_bf = du.astype(jnp.bfloat16)
        dw1_acc[...] += _tn(dg_bf, n2_bf)
        dw3_acc[...] += _tn(du_bf, n2_bf)
        dn2 = _nt(dg_bf, w1_ref[...]) + _nt(du_bf, w3_ref[...])
        dh = G32 + _ln_bwd(dn2, n2, r2)
        da = dh.astype(jnp.bfloat16)
        dwo_acc[...] += _nn(o_bf, da)
        dot_s[...] = _nt(wo_ref[...], da).astype(jnp.bfloat16)
        dh_s[rows, :] = dh

    with _scope('attn_bwd'):
        def dpk(h, s_ref):
            doT = dot_s[pl.ds(pl.multiple_of(h * Dh, Dh), Dh), :]
            s_ref[...] = _nn(v_s[...], doT)

        def fused_bwd(hn, sn_ref, h, s_ref):
            hs = pl.multiple_of(h * Dh, Dh)
            doTn = dot_s[pl.ds(pl.multiple_of(hn * Dh, Dh), Dh), :]
            qt = qt_s[pl.ds(hs, Dh), :].astype(jnp.float32)
            doT = dot_s[pl.ds(hs, Dh), :].astype(jnp.float32)
            oT = ot_s[pl.ds(hs, Dh), :]
            delta = jnp.sum(doT * oT, axis=0, keepdims=True)
            linv = l_s[h]
            qtl = (qt * linv).astype(jnp.bfloat16)
            dol = (doT * linv).astype(jnp.bfloat16)
            dqT = jnp.zeros((Dh, BQ), jnp.float32)
            for c in range(NC):
                ks = slice(c * CK, (c + 1) * CK)
                sn_ref[ks, :] = _nn(v_s[ks, :], doTn)
                pb = p_s[h, ks, :]
                ds = (pb.astype(jnp.float32) * (s_ref[ks, :] - delta)).astype(jnp.bfloat16)
                dqT = dqT + _nn(kt_s[:, ks], ds)
                dkt_s[:, ks] += _nt(qtl, ds)
                dvt_s[:, ks] += _nt(dol, pb)
            dqt_s[pl.ds(hs, Dh), :] = dqT * (linv * SCALE)

        dpk(0, s_a)

        def bwd_body(j, c):
            h0 = 2 * j; h1 = 2 * j + 1
            hn = jnp.minimum(h1 + 1, H - 1)
            fused_bwd(h1, s_b, h0, s_a)
            fused_bwd(hn, s_a, h1, s_b)
            return c
        jax.lax.fori_loop(0, H // 2, bwd_body, 0)

    with _scope('wgrad_q'):
        dqt_bf = dqt_s[...].astype(jnp.bfloat16)
        dwqt_acc[...] += _nn(dqt_bf, n1_blk)
        dn1_s[rows, :] = jax.lax.dot_general(dqt_bf, wq_ref[...], (((0,), (1,)), ((), ())), preferred_element_type=jnp.float32)

    with _scope('epilogue'):
        @pl.when(i == NQ - 1)
        def _():
            dkt_bf = dkt_s[...].astype(jnp.bfloat16)
            dvt_bf = dvt_s[...].astype(jnp.bfloat16)
            def dx_chunk(c, carry):
                rs = pl.ds(pl.multiple_of(c * BQ, BQ), BQ)
                n = n1_s[rs, :].astype(jnp.float32)
                dn = dn1_s[rs, :] + dn1_kv_chunk(c)
                dx_ref[rs, :] = (dh_s[rs, :] + _ln_bwd(dn, n, r1_s[rs, :])).astype(dx_ref.dtype)
                return carry

            def dn1_kv_chunk(c):
                cs = pl.ds(pl.multiple_of(c * BQ, BQ), BQ)
                dk = dkt_s[:, cs].astype(jnp.bfloat16)
                dv = dvt_s[:, cs].astype(jnp.bfloat16)
                return jax.lax.dot_general(dk, wk_ref[...], (((0,), (1,)), ((), ())),
                                           preferred_element_type=jnp.float32) + \
                       jax.lax.dot_general(dv, wv_ref[...], (((0,), (1,)), ((), ())),
                                           preferred_element_type=jnp.float32)
            for c in range(NQ):
                dx_chunk(c, 0)
            dwk_ref[...] = _nn(dkt_bf, n1_s[...]).astype(dwk_ref.dtype)
            dwv_ref[...] = _nn(dvt_bf, n1_s[...]).astype(dwv_ref.dtype)
            dwq_ref[...] = dwqt_acc[...].T.astype(dwq_ref.dtype)
            dwo_ref[...] = dwo_acc[...].astype(dwo_ref.dtype)
            dw1_ref[...] = dw1_acc[...].astype(dw1_ref.dtype)
            dw3_ref[...] = dw3_acc[...].astype(dw3_ref.dtype)
            dw2_ref[...] = dw2_acc[...].astype(dw2_ref.dtype)


@jax.jit
def pallas_sequential_preLN__grouped_kv_mqa__glu_gated_swiglu__prompt_kernel(
    A_x: jax.Array,
    A_wq: jax.Array,
    A_wk: jax.Array,
    A_wv: jax.Array,
    A_wo: jax.Array,
    B_x: jax.Array,
    B_w1: jax.Array,
    B_w3: jax.Array,
    B_w2: jax.Array,
    grad_out: jax.Array,
):
    x = A_x.reshape(S, D)
    g = grad_out.reshape(S, D)
    full = lambda shape: pl.BlockSpec(shape, lambda i: (0,) * len(shape), pipeline_mode=pl.Buffered(1))
    bf = jnp.bfloat16
    f32 = jnp.float32
    out_shape = [
        jax.ShapeDtypeStruct((S, D), bf),
        jax.ShapeDtypeStruct((S, D), bf),
        jax.ShapeDtypeStruct((D, H * Dh), bf),
        jax.ShapeDtypeStruct((Dh, D), bf),
        jax.ShapeDtypeStruct((Dh, D), bf),
        jax.ShapeDtypeStruct((H * Dh, D), bf),
        jax.ShapeDtypeStruct((F, D), bf),
        jax.ShapeDtypeStruct((F, D), bf),
        jax.ShapeDtypeStruct((F, D), bf),
    ]
    fullout = lambda shape: pl.BlockSpec(shape, lambda i: (0,) * len(shape))
    outs = pl.pallas_call(
        _kernel,
        grid=(NQ,),
        in_specs=[
            full((S, D)), full((S, D)), full((D, H * Dh)), full((D, Dh)), full((D, Dh)),
            full((H * Dh, D)), full((D, F)), full((D, F)), full((F, D)),
        ],
        out_specs=[
            pl.BlockSpec((BQ, D), lambda i: (i, 0)),
            fullout((S, D)), fullout((D, H * Dh)), fullout((Dh, D)), fullout((Dh, D)),
            fullout((H * Dh, D)), fullout((F, D)), fullout((F, D)), fullout((F, D)),
        ],
        out_shape=out_shape,
        scratch_shapes=[
            pltpu.VMEM((S, D), bf),
            pltpu.VMEM((S, 1), f32),
            pltpu.VMEM((S, D), f32),
            pltpu.VMEM((S, D), f32),
            pltpu.VMEM((S, Dh), bf),
            pltpu.VMEM((S, Dh), bf),
            pltpu.VMEM((Dh, S), bf),
            pltpu.VMEM((Dh, S), bf),
            pltpu.VMEM((H * Dh, D), bf),
            pltpu.VMEM((H * Dh, BQ), bf),
            pltpu.VMEM((H * Dh, BQ), f32),
            pltpu.VMEM((H * Dh, BQ), bf),
            pltpu.VMEM((H * Dh, BQ), f32),
            pltpu.VMEM((H, S, BQ), bf),
            pltpu.VMEM((S, BQ), f32),
            pltpu.VMEM((S, BQ), f32),
            pltpu.VMEM((1, BQ), f32),
            pltpu.VMEM((1, BQ), f32),
            pltpu.VMEM((H, 1, BQ), f32),
            pltpu.VMEM((Dh, S), f32),
            pltpu.VMEM((Dh, S), f32),
            pltpu.VMEM((H * Dh, D), f32),
            pltpu.VMEM((H * Dh, D), f32),
            pltpu.VMEM((F, D), f32),
            pltpu.VMEM((F, D), f32),
            pltpu.VMEM((F, D), f32),
        ],
        compiler_params=pltpu.CompilerParams(
            dimension_semantics=("arbitrary",),
            vmem_limit_bytes=110 * 1024 * 1024,
        ),
    )(x, g, A_wq, A_wk, A_wv, A_wo, B_w1, B_w3, B_w2)
    out, dx, dwq, dwk, dwv, dwo, dw1, dw3, dw2 = outs
    return (out.reshape(1, S, D), dx.reshape(1, S, D), dwq, dwk.T, dwv.T, dwo, dw1.T, dw3.T, dw2)
```
